```python
import jax
import jax.numpy as jnp

def _softmax(x, axis=-1):
    return jax.nn.softmax(x, axis=axis)
def _gelu(x):
    return jax.nn.gelu(x, approximate=True)
def _silu(x):
    return jax.nn.silu(x)
def _sigmoid(x):
    return jax.nn.sigmoid(x)
def _layernorm(x, axis=-1, eps=1e-5):
    m = jnp.mean(x, axis=axis, keepdims=True)
    v = jnp.var(x, axis=axis, keepdims=True)
    return (x - m) / jnp.sqrt(v + eps)
def _scatter_add(tgt, idx, src, axis=0):
    return tgt.at[idx].add(src)
def _segment_sum(src, seg, n):
    return jax.ops.segment_sum(src, seg, n)
class _Rng:
    def __init__(self, key):
        self._k = key
    def _next(self):
        self._k, sub = jax.random.split(self._k)
        return sub
    def normal(self, shape):
        return jax.random.normal(self._next(), shape, dtype=jnp.bfloat16)
    def randint(self, lo, hi, shape):
        return jax.random.randint(self._next(), shape, lo, hi, dtype=jnp.int32)
    def uniform(self, shape, lo=0.0, hi=1.0):
        return jax.random.uniform(self._next(), shape, jnp.bfloat16, lo, hi)
    def permutation(self, n):
        return jax.random.permutation(self._next(), n)


kernel_name = 'standalone__standard_2d_1d_3d_conv__vision'

def setup_inputs():
    _rng = _Rng(jax.random.key(int.from_bytes(__import__("os").urandom(4), "little")))
    _w = (lambda a: (lambda t: t.astype(jnp.bfloat16) if jnp.issubdtype(t.dtype, jnp.floating) else t)(jnp.asarray(a)))
    H = W = 384
    C = 384
    K = 1
    return {
        "x": _w((lambda *s: _rng.normal(s) * 0.05)(1, H, W, C)),
        "w": _w((lambda *s: _rng.normal(s) * 0.05)(K, K, C, C)),
        "b": _w((lambda *s: _rng.normal(s) * 0.05)(C)),
    }

def reference(x, w, b):
    B, H, W, Cin = x.shape
    K = w.shape[0]
    pl = (K - 1) // 2
    pr = K // 2
    xp = jnp.pad(x, ((0, 0), (pl, pr), (pl, pr), (0, 0)))
    out = sum(
        jnp.einsum('bhwc,cd->bhwd', xp[:, i:i+H, j:j+W, :], w[i, j])
        for i in range(K) for j in range(K)
    )
    return out + b[None, None, None, :]
```

```python
import jax
import jax.numpy as jnp
import jax.experimental.pallas as pl
import jax.experimental.pallas.tpu as pltpu

_SLAB = 2048
_STREAMS = 8
_PIECE = 16
_READ_SLABS = 2
_SWITCH = 43
_BURST = 64
_PER_TILE = 32
_LAST = 512


def _make_kernel(n_slabs, c_out):
    n_pieces = _SLAB // _PIECE
    n_writes = (n_slabs // _STREAMS) * n_pieces
    n_reads = n_slabs // _READ_SLABS
    n_late = n_slabs - _SWITCH
    rest = n_writes - _BURST - n_late * _PER_TILE

    def writes_ready(tiles_done):
        return (tiles_done // _STREAMS) * n_pieces

    assert n_slabs % _STREAMS == 0 and n_slabs % _READ_SLABS == 0
    assert _READ_SLABS > 1 and rest >= 0 and _BURST <= writes_ready(_SWITCH)
    for j in range(_SWITCH, n_slabs):
        assert _BURST + (j - _SWITCH + 1) * _PER_TILE <= writes_ready(j + 1)

    def kernel(x_hbm, w_hbm, b_hbm, o_hbm, buf, w_v, b_v, bias_v,
               read_sem, par_sem, write_sem):
        def read(c):
            rows = pl.ds(c * _READ_SLABS, _READ_SLABS)
            return pltpu.make_async_copy(x_hbm.at[rows], buf.at[rows], read_sem.at[c])

        def read_part(idx, sem_id):
            return pltpu.make_async_copy(x_hbm.at[idx], buf.at[idx], read_sem.at[sem_id])

        def write(i):
            idx = (
                pl.ds((i // n_pieces) * _STREAMS, _STREAMS),
                pl.ds(pl.multiple_of((i % n_pieces) * _PIECE, _PIECE), _PIECE),
                slice(None),
            )
            return pltpu.make_async_copy(buf.at[idx], o_hbm.at[idx], write_sem.at[0])

        def queue_writes(first, count):
            def body(i, carry):
                write(first + i).start()
                return carry
            jax.lax.fori_loop(0, count, body, 0)

        def compute(j):
            acc = jnp.dot(buf[j], w_v[0, 0], preferred_element_type=jnp.float32)
            buf[j] = (acc + bias_v[0:1, :]).astype(buf.dtype)

        w_copy = pltpu.make_async_copy(w_hbm, w_v, par_sem.at[0])
        b_copy = pltpu.make_async_copy(b_hbm, b_v, par_sem.at[1])
        last = n_reads - 1
        tail_a = read_part((pl.ds(last * _READ_SLABS, _READ_SLABS - 1),), last)
        tail_b = read_part((n_slabs - 1, pl.ds(0, _SLAB - _LAST)), last + 1)
        tail_c = read_part((n_slabs - 1, pl.ds(_SLAB - _LAST, _LAST)), last + 2)

        w_copy.start()
        b_copy.start()

        def start_read(c, carry):
            read(c).start()
            return carry
        jax.lax.fori_loop(0, last, start_read, 0)
        tail_a.start()
        tail_b.start()
        tail_c.start(priority=1)

        w_copy.wait()
        b_copy.wait()
        bias_v[...] = jnp.broadcast_to(
            b_v[...].astype(jnp.float32).reshape(1, c_out), bias_v.shape)

        def early(j, carry):
            @pl.when(j % _READ_SLABS == 0)
            def _():
                read(j // _READ_SLABS).wait()
            compute(j)
            return carry
        jax.lax.fori_loop(0, _SWITCH, early, 0)

        for c in range(pl.cdiv(_SWITCH, _READ_SLABS), last):
            read(c).wait()
        tail_a.wait()
        tail_b.wait()
        queue_writes(0, _BURST)
        tail_c.wait()

        def late(j, carry):
            compute(j)
            queue_writes(_BURST + (j - _SWITCH) * _PER_TILE, _PER_TILE)
            return carry
        jax.lax.fori_loop(_SWITCH, n_slabs, late, 0)
        if rest:
            queue_writes(n_writes - rest, rest)
        pltpu.make_async_copy(buf, o_hbm, write_sem.at[0]).wait()

    return kernel, n_reads


@jax.jit
def pallas_standalone__standard_2d_1d_3d_conv__vision_kernel(
    x: jax.Array,
    w: jax.Array,
    b: jax.Array,
):
    n, h, wd, c_in = x.shape
    c_out = w.shape[3]
    assert w.shape[:2] == (1, 1) and c_in == c_out
    rows = n * h * wd
    n_slabs = rows // _SLAB
    assert n_slabs * _SLAB == rows
    kernel, n_reads = _make_kernel(n_slabs, c_out)
    out = pl.pallas_call(
        kernel,
        in_specs=[pl.BlockSpec(memory_space=pl.ANY)] * 3,
        out_specs=pl.BlockSpec(memory_space=pl.ANY),
        out_shape=jax.ShapeDtypeStruct((n_slabs, _SLAB, c_out), x.dtype),
        scratch_shapes=[
            pltpu.VMEM((n_slabs, _SLAB, c_in), x.dtype),
            pltpu.VMEM(w.shape, w.dtype),
            pltpu.VMEM(b.shape, b.dtype),
            pltpu.VMEM((8, c_out), jnp.float32),
            pltpu.SemaphoreType.DMA((n_reads + 2,)),
            pltpu.SemaphoreType.DMA((2,)),
            pltpu.SemaphoreType.DMA((1,)),
        ],
        compiler_params=pltpu.CompilerParams(vmem_limit_bytes=120 * 1024 * 1024),
    )(x.reshape(n_slabs, _SLAB, c_in), w, b)
    return out.reshape(n, h, wd, c_out)
```

```python
import functools

import jax
import jax.numpy as jnp
import jax.experimental.pallas as pl
import jax.experimental.pallas.tpu as pltpu

_SLAB = 2048
_STREAMS = 6
_PIECE = 16
_TILE = 256
_SUB = 128
_LEAD = 3
_EXTRA = 1
_RD_CHUNK = 4
_TAIL_CHUNKS = 2
_WR_CHUNK = 2
_BURST = 36
_PER_TILE = 14


def _log2(n):
    assert n & (n - 1) == 0
    return n.bit_length() - 1


def _make_kernel(n_slabs, c_out):
    tiles_per_group = _SLAB // _TILE
    n_tiles = (n_slabs // _STREAMS) * tiles_per_group
    half = n_tiles // 2
    rd_chunks = _TILE // (_PIECE * _RD_CHUNK)
    wr_chunks = _TILE // (_PIECE * _WR_CHUNK)
    n_early = half - _LEAD + _EXTRA
    rest = n_tiles * wr_chunks - _BURST - (n_tiles - n_early) * _PER_TILE
    tail_rows = _TAIL_CHUNKS * _RD_CHUNK * _PIECE

    assert n_slabs % (2 * _STREAMS) == 0 and _EXTRA <= _LEAD < half
    assert rest >= 0 and tail_rows < _TILE
    assert _BURST <= n_early * wr_chunks
    for j in range(n_early, n_tiles):
        assert _BURST + (j - n_early + 1) * _PER_TILE <= (j + 1) * wr_chunks

    def window(t, row, rows):
        if isinstance(t, int):
            group = t // tiles_per_group
        else:
            group = jax.lax.shift_right_logical(t, _log2(tiles_per_group))
        start = (t & (tiles_per_group - 1)) * _TILE + row
        if not isinstance(start, int):
            start = pl.multiple_of(start, _PIECE)
        return (pl.ds(group * _STREAMS, _STREAMS), pl.ds(start, rows), slice(None))

    def kernel(x_hbm, w_hbm, b_hbm, o_hbm, buf, w_v, b_v, bias_v,
               read_sem, par_sem, write_sem):
        def read(t, row, rows, sem_id):
            idx = window(t, row, rows)
            return pltpu.make_async_copy(x_hbm.at[idx], buf.at[idx], read_sem.at[sem_id])

        def queue_reads(t, final=False):
            def chunk(c, carry, low_sem):
                for q in range(_RD_CHUNK):
                    row = (c * _RD_CHUNK + q) * _PIECE
                    read(t, row, _PIECE, t).start(priority=0)
                    read(t + half, row, _PIECE, low_sem).start(priority=1)
                return carry
            split = rd_chunks - _TAIL_CHUNKS if final else rd_chunks
            jax.lax.fori_loop(0, split, functools.partial(chunk, low_sem=t + half), 0)
            if final:
                jax.lax.fori_loop(
                    split, rd_chunks, functools.partial(chunk, low_sem=n_tiles), 0)

        def queue_writes(first, count):
            def body(i, carry):
                c = first + i
                t = jax.lax.shift_right_logical(c, _log2(wr_chunks))
                row = (c & (wr_chunks - 1)) * (_WR_CHUNK * _PIECE)
                for q in range(_WR_CHUNK):
                    idx = window(t, row + q * _PIECE, _PIECE)
                    pltpu.make_async_copy(
                        buf.at[idx], o_hbm.at[idx], write_sem.at[0]).start()
                return carry
            jax.lax.fori_loop(0, count, body, 0)

        def compute(t):
            tile = buf.at[window(t, 0, _TILE)]
            for s in range(_STREAMS):
                for q in range(_TILE // _SUB):
                    rows = pl.ds(q * _SUB, _SUB)
                    acc = jnp.dot(tile[s, rows, :], w_v[0, 0],
                                  preferred_element_type=jnp.float32)
                    tile[s, rows, :] = (acc + bias_v[0:1, :]).astype(buf.dtype)

        w_copy = pltpu.make_async_copy(w_hbm, w_v, par_sem.at[0])
        b_copy = pltpu.make_async_copy(b_hbm, b_v, par_sem.at[1])

        w_copy.start()
        b_copy.start()

        def prologue(t, carry):
            queue_reads(t)
            return carry
        jax.lax.fori_loop(0, _LEAD, prologue, 0)

        w_copy.wait()
        b_copy.wait()
        bias_v[...] = jnp.broadcast_to(
            b_v[...].astype(jnp.float32).reshape(1, c_out), bias_v.shape)

        def early(j, carry):
            read(j, 0, _TILE, j).wait()
            compute(j)

            @pl.when(j + _LEAD < half - 1)
            def _():
                queue_reads(j + _LEAD)

            @pl.when(j + _LEAD == half - 1)
            def _():
                queue_reads(half - 1, final=True)
            return carry
        jax.lax.fori_loop(0, n_early, early, 0)

        def drain(t, carry):
            read(t, 0, _TILE, t).wait()
            return carry
        jax.lax.fori_loop(n_early, n_tiles - 1, drain, 0)
        read(n_tiles - 1, 0, _TILE - tail_rows, n_tiles - 1).wait()
        queue_writes(0, _BURST)
        read(n_tiles - 1, _TILE - tail_rows, tail_rows, n_tiles).wait()

        def late(j, carry):
            compute(j)
            queue_writes(_BURST + (j - n_early) * _PER_TILE, _PER_TILE)
            return carry
        jax.lax.fori_loop(n_early, n_tiles, late, 0)
        if rest:
            queue_writes(n_tiles * wr_chunks - rest, rest)
        pltpu.make_async_copy(buf, o_hbm, write_sem.at[0]).wait()

    return kernel, n_tiles


@jax.jit
def pallas_standalone__standard_2d_1d_3d_conv__vision_kernel(
    x: jax.Array,
    w: jax.Array,
    b: jax.Array,
):
    n, h, wd, c_in = x.shape
    c_out = w.shape[3]
    assert w.shape[:2] == (1, 1) and c_in == c_out
    rows = n * h * wd
    n_slabs = rows // _SLAB
    assert n_slabs * _SLAB == rows
    kernel, n_tiles = _make_kernel(n_slabs, c_out)
    out = pl.pallas_call(
        kernel,
        in_specs=[pl.BlockSpec(memory_space=pl.ANY)] * 3,
        out_specs=pl.BlockSpec(memory_space=pl.ANY),
        out_shape=jax.ShapeDtypeStruct((n_slabs, _SLAB, c_out), x.dtype),
        scratch_shapes=[
            pltpu.VMEM((n_slabs, _SLAB, c_in), x.dtype),
            pltpu.VMEM(w.shape, w.dtype),
            pltpu.VMEM(b.shape, b.dtype),
            pltpu.VMEM((8, c_out), jnp.float32),
            pltpu.SemaphoreType.DMA((n_tiles + 1,)),
            pltpu.SemaphoreType.DMA((2,)),
            pltpu.SemaphoreType.DMA((1,)),
        ],
        compiler_params=pltpu.CompilerParams(
            vmem_limit_bytes=120 * 1024 * 1024,
            disable_bounds_checks=True,
        ),
    )(x.reshape(n_slabs, _SLAB, c_in), w, b)
    return out.reshape(n, h, wd, c_out)
```

```python
import jax
import jax.numpy as jnp
import jax.experimental.pallas as pl
import jax.experimental.pallas.tpu as pltpu

_SLAB = 2048
_STREAMS = 6
_TILE = 256
_SUB = 128
_RD_ROWS = 8
_RD_UNROLL = 4
_RD_PARTS = 2
_LEAD = 2
_TAIL = 3
_WR_ROWS = 16
_WR_UNROLL = 4
_BURST = 16
_PER_TILE = 7

_RING = 4
_SEM_LOW, _SEM_TAIL, _SEM_W, _SEM_B, _SEM_OUT = range(_RING, _RING + 5)


def _log2(n):
    assert n & (n - 1) == 0
    return n.bit_length() - 1


def _make_kernel(n_slabs, c_out):
    tiles_per_group = _SLAB // _TILE
    n_tiles = (n_slabs // _STREAMS) * tiles_per_group
    half = n_tiles // 2
    rd_rows = _RD_ROWS * _RD_UNROLL
    wr_rows = _WR_ROWS * _WR_UNROLL
    rd_chunks = _TILE // rd_rows
    wr_chunks = _TILE // wr_rows
    n_early = half - _LEAD
    rest = n_tiles * wr_chunks - _BURST - (n_tiles - n_early) * _PER_TILE
    tail_rows = _TAIL * rd_rows

    assert n_slabs % (2 * _STREAMS) == 0 and _LEAD < _RING and _LEAD < half
    assert rd_chunks % _RD_PARTS == 0 and _STREAMS % _RD_PARTS == 0
    assert rd_chunks * rd_rows == _TILE and wr_chunks * wr_rows == _TILE
    assert rest >= 0 and 0 < _TAIL <= rd_chunks // _RD_PARTS
    assert _BURST <= n_early * wr_chunks
    for j in range(n_early, n_tiles):
        assert _BURST + (j - n_early + 1) * _PER_TILE <= (j + 1) * wr_chunks

    def window(t, row, rows):
        if isinstance(t, int):
            group = t // tiles_per_group
        else:
            group = jax.lax.shift_right_logical(t, _log2(tiles_per_group))
        start = (t & (tiles_per_group - 1)) * _TILE + row
        if not isinstance(start, int):
            start = pl.multiple_of(start, _RD_ROWS)
        return (pl.ds(group * _STREAMS, _STREAMS), pl.ds(start, rows), slice(None))

    def kernel(x_hbm, w_hbm, b_hbm, o_hbm, buf, w_v, b_v, bias_v, sem):
        def read(idx, sem_id):
            return pltpu.make_async_copy(x_hbm.at[idx], buf.at[idx], sem.at[sem_id])

        def queue_reads(t, first, stop, low_sem):
            def chunk(c, carry):
                hi = window(t, c * rd_rows, rd_rows)
                lo = window(t + half, c * rd_rows, rd_rows)
                x_hi, buf_hi, x_lo, buf_lo = (
                    x_hbm.at[hi], buf.at[hi], x_hbm.at[lo], buf.at[lo])
                for q in range(_RD_UNROLL):
                    rows = (slice(None), pl.ds(q * _RD_ROWS, _RD_ROWS))
                    pltpu.make_async_copy(
                        x_hi.at[rows], buf_hi.at[rows], sem.at[t & (_RING - 1)]
                    ).start(priority=0)
                    pltpu.make_async_copy(
                        x_lo.at[rows], buf_lo.at[rows], sem.at[low_sem]
                    ).start(priority=1)
                return carry
            if stop > first:
                jax.lax.fori_loop(first, stop, chunk, 0)

        def queue_writes(first, count):
            def chunk(i, carry):
                c = first + i
                t = jax.lax.shift_right_logical(c, _log2(wr_chunks))
                idx = window(t, (c & (wr_chunks - 1)) * wr_rows, wr_rows)
                src, dst = buf.at[idx], o_hbm.at[idx]
                for q in range(_WR_UNROLL):
                    rows = (slice(None), pl.ds(q * _WR_ROWS, _WR_ROWS))
                    pltpu.make_async_copy(
                        src.at[rows], dst.at[rows], sem.at[_SEM_OUT]).start()
                return carry
            jax.lax.fori_loop(0, count, chunk, 0)

        def compute(t, first_slab, stop_slab):
            tile = buf.at[window(t, 0, _TILE)]
            for s in range(first_slab, stop_slab):
                for q in range(_TILE // _SUB):
                    rows = pl.ds(q * _SUB, _SUB)
                    acc = jnp.dot(tile[s, rows, :], w_v[0, 0],
                                  preferred_element_type=jnp.float32)
                    tile[s, rows, :] = (acc + bias_v[0:1, :]).astype(buf.dtype)

        w_copy = pltpu.make_async_copy(w_hbm, w_v, sem.at[_SEM_W])
        b_copy = pltpu.make_async_copy(b_hbm, b_v, sem.at[_SEM_B])

        w_copy.start()
        b_copy.start()

        def prologue(t, carry):
            queue_reads(t, 0, rd_chunks, _SEM_LOW)
            return carry
        jax.lax.fori_loop(0, _LEAD, prologue, 0)

        w_copy.wait()
        b_copy.wait()
        bias_v[...] = jnp.broadcast_to(
            b_v[...].astype(jnp.float32).reshape(1, c_out), bias_v.shape)

        def early(j, carry):
            read(window(j, 0, _TILE), j & (_RING - 1)).wait()
            for p in range(_RD_PARTS):
                compute(j, p * _STREAMS // _RD_PARTS, (p + 1) * _STREAMS // _RD_PARTS)
                first = p * rd_chunks // _RD_PARTS
                stop = (p + 1) * rd_chunks // _RD_PARTS
                if p < _RD_PARTS - 1:
                    queue_reads(j + _LEAD, first, stop, _SEM_LOW)
                else:
                    queue_reads(j + _LEAD, first, stop - _TAIL, _SEM_LOW)
                    low_sem = jnp.where(j == n_early - 1, _SEM_TAIL, _SEM_LOW)
                    queue_reads(j + _LEAD, stop - _TAIL, stop, low_sem)
            return carry
        jax.lax.fori_loop(0, n_early, early, 0)

        for t in range(n_early, half):
            read(window(t, 0, _TILE), t & (_RING - 1)).wait()
        read((pl.ds(n_slabs // 2, n_slabs // 2 - _STREAMS),), _SEM_LOW).wait()
        read((pl.ds(n_slabs - _STREAMS, _STREAMS), pl.ds(0, _SLAB - tail_rows)),
             _SEM_LOW).wait()
        queue_writes(0, _BURST)
        read(window(n_tiles - 1, _TILE - tail_rows, tail_rows), _SEM_TAIL).wait()

        def late(j, carry):
            compute(j, 0, _STREAMS)
            queue_writes(_BURST + (j - n_early) * _PER_TILE, _PER_TILE)
            return carry
        jax.lax.fori_loop(n_early, n_tiles, late, 0)
        if rest:
            queue_writes(n_tiles * wr_chunks - rest, rest)
        pltpu.make_async_copy(buf, o_hbm, sem.at[_SEM_OUT]).wait()

    return kernel


@jax.jit
def pallas_standalone__standard_2d_1d_3d_conv__vision_kernel(
    x: jax.Array,
    w: jax.Array,
    b: jax.Array,
):
    n, h, wd, c_in = x.shape
    c_out = w.shape[3]
    assert w.shape[:2] == (1, 1) and c_in == c_out
    rows = n * h * wd
    n_slabs = rows // _SLAB
    assert n_slabs * _SLAB == rows
    out = pl.pallas_call(
        _make_kernel(n_slabs, c_out),
        in_specs=[pl.BlockSpec(memory_space=pl.ANY)] * 3,
        out_specs=pl.BlockSpec(memory_space=pl.ANY),
        out_shape=jax.ShapeDtypeStruct((n_slabs, _SLAB, c_out), x.dtype),
        scratch_shapes=[
            pltpu.VMEM((n_slabs, _SLAB, c_in), x.dtype),
            pltpu.VMEM(w.shape, w.dtype),
            pltpu.VMEM(b.shape, b.dtype),
            pltpu.VMEM((8, c_out), jnp.float32),
            pltpu.SemaphoreType.DMA((_SEM_OUT + 1,)),
        ],
        compiler_params=pltpu.CompilerParams(
            vmem_limit_bytes=120 * 1024 * 1024,
            disable_bounds_checks=True,
            disable_semaphore_checks=True,
        ),
    )(x.reshape(n_slabs, _SLAB, c_in), w, b)
    return out.reshape(n, h, wd, c_out)
```

```python
import jax
import jax.numpy as jnp
import jax.experimental.pallas as pl
import jax.experimental.pallas.tpu as pltpu

_SLAB = 2048
_STREAMS = 6
_TILE = 256
_SUB = 128
_RD_ROWS = 8
_RD_UNROLL = 4
_RD_PARTS = 2
_LEAD = 2
_TAIL = 3
_WR_ROWS = 16
_WR_UNROLL = 4
_BURST = 16
_PER_TILE = 7

_RING = 4
_SEM_LOW, _SEM_TAIL, _SEM_W, _SEM_B, _SEM_OUT = range(_RING, _RING + 5)


def _log2(n):
    assert n & (n - 1) == 0
    return n.bit_length() - 1


def _make_kernel(n_slabs, c_out):
    tiles_per_group = _SLAB // _TILE
    n_tiles = (n_slabs // _STREAMS) * tiles_per_group
    half = n_tiles // 2
    rd_rows = _RD_ROWS * _RD_UNROLL
    wr_rows = _WR_ROWS * _WR_UNROLL
    rd_chunks = _TILE // rd_rows
    wr_chunks = _TILE // wr_rows
    n_early = half - _LEAD
    rest = n_tiles * wr_chunks - _BURST - (n_tiles - n_early) * _PER_TILE
    tail_rows = _TAIL * rd_rows

    assert n_slabs % (2 * _STREAMS) == 0 and _LEAD < _RING and _LEAD < half
    assert rd_chunks % _RD_PARTS == 0 and _STREAMS % _RD_PARTS == 0
    assert rd_chunks * rd_rows == _TILE and wr_chunks * wr_rows == _TILE
    assert rest >= 0 and 0 < _TAIL <= rd_chunks // _RD_PARTS
    assert _BURST <= n_early * wr_chunks
    for j in range(n_early, n_tiles):
        assert _BURST + (j - n_early + 1) * _PER_TILE <= (j + 1) * wr_chunks

    def window(t, row, rows):
        if isinstance(t, int):
            group = t // tiles_per_group
        else:
            group = jax.lax.shift_right_logical(t, _log2(tiles_per_group))
        start = (t & (tiles_per_group - 1)) * _TILE + row
        if not isinstance(start, int):
            start = pl.multiple_of(start, _RD_ROWS)
        return (pl.ds(group * _STREAMS, _STREAMS), pl.ds(start, rows), slice(None))

    def kernel(x_hbm, w_hbm, b_hbm, o_hbm, buf, w_v, b_v, bias_v, sem):
        def read(idx, sem_id):
            return pltpu.make_async_copy(x_hbm.at[idx], buf.at[idx], sem.at[sem_id])

        def queue_reads(t, first, stop, low_sem):
            def chunk(c, carry):
                hi = window(t, c * rd_rows, rd_rows)
                lo = window(t + half, c * rd_rows, rd_rows)
                x_hi, buf_hi, x_lo, buf_lo = (
                    x_hbm.at[hi], buf.at[hi], x_hbm.at[lo], buf.at[lo])
                for q in range(_RD_UNROLL):
                    rows = (slice(None), pl.ds(q * _RD_ROWS, _RD_ROWS))
                    pltpu.make_async_copy(
                        x_hi.at[rows], buf_hi.at[rows], sem.at[t & (_RING - 1)]
                    ).start(priority=0)
                    pltpu.make_async_copy(
                        x_lo.at[rows], buf_lo.at[rows], sem.at[low_sem]
                    ).start(priority=1)
                return carry
            if stop > first:
                jax.lax.fori_loop(first, stop, chunk, 0)

        def queue_writes(first, count):
            def chunk(i, carry):
                c = first + i
                t = jax.lax.shift_right_logical(c, _log2(wr_chunks))
                idx = window(t, (c & (wr_chunks - 1)) * wr_rows, wr_rows)
                src, dst = buf.at[idx], o_hbm.at[idx]
                for q in range(_WR_UNROLL):
                    rows = (slice(None), pl.ds(q * _WR_ROWS, _WR_ROWS))
                    pltpu.make_async_copy(
                        src.at[rows], dst.at[rows], sem.at[_SEM_OUT]).start()
                return carry
            jax.lax.fori_loop(0, count, chunk, 0)

        def compute(t, first_slab, stop_slab):
            tile = buf.at[window(t, 0, _TILE)]
            for s in range(first_slab, stop_slab):
                for q in range(_TILE // _SUB):
                    rows = pl.ds(q * _SUB, _SUB)
                    acc = jnp.dot(tile[s, rows, :], w_v[0, 0],
                                  preferred_element_type=jnp.float32)
                    tile[s, rows, :] = (acc + bias_v[0:1, :]).astype(buf.dtype)

        w_copy = pltpu.make_async_copy(w_hbm, w_v, sem.at[_SEM_W])
        b_copy = pltpu.make_async_copy(b_hbm, b_v, sem.at[_SEM_B])

        w_copy.start()
        b_copy.start()

        def prologue(t, carry):
            queue_reads(t, 0, rd_chunks, _SEM_LOW)
            return carry
        jax.lax.fori_loop(0, _LEAD, prologue, 0)

        w_copy.wait()
        b_copy.wait()
        bias_v[...] = jnp.broadcast_to(
            b_v[...].astype(jnp.float32).reshape(1, c_out), bias_v.shape)

        def early(j, carry):
            read(window(j, 0, _TILE), j & (_RING - 1)).wait()
            for p in range(_RD_PARTS):
                compute(j, p * _STREAMS // _RD_PARTS, (p + 1) * _STREAMS // _RD_PARTS)
                first = p * rd_chunks // _RD_PARTS
                stop = (p + 1) * rd_chunks // _RD_PARTS
                if p < _RD_PARTS - 1:
                    queue_reads(j + _LEAD, first, stop, _SEM_LOW)
                else:
                    queue_reads(j + _LEAD, first, stop - _TAIL, _SEM_LOW)

                    @pl.when(j < n_early - 1)
                    def _():
                        queue_reads(j + _LEAD, stop - _TAIL, stop, _SEM_LOW)
            return carry
        jax.lax.fori_loop(0, n_early, early, 0)
        queue_reads(half - 1, rd_chunks - _TAIL, rd_chunks, _SEM_TAIL)

        for t in range(n_early, half):
            read(window(t, 0, _TILE), t & (_RING - 1)).wait()
        read((pl.ds(n_slabs // 2, n_slabs // 2 - _STREAMS),), _SEM_LOW).wait()
        read((pl.ds(n_slabs - _STREAMS, _STREAMS), pl.ds(0, _SLAB - tail_rows)),
             _SEM_LOW).wait()
        queue_writes(0, _BURST)
        read(window(n_tiles - 1, _TILE - tail_rows, tail_rows), _SEM_TAIL).wait()

        def late(j, carry):
            compute(j, 0, _STREAMS)
            queue_writes(_BURST + (j - n_early) * _PER_TILE, _PER_TILE)
            return carry
        jax.lax.fori_loop(n_early, n_tiles, late, 0)
        if rest:
            queue_writes(n_tiles * wr_chunks - rest, rest)
        pltpu.make_async_copy(buf, o_hbm, sem.at[_SEM_OUT]).wait()

    return kernel


@jax.jit
def pallas_standalone__standard_2d_1d_3d_conv__vision_kernel(
    x: jax.Array,
    w: jax.Array,
    b: jax.Array,
):
    n, h, wd, c_in = x.shape
    c_out = w.shape[3]
    assert w.shape[:2] == (1, 1) and c_in == c_out
    rows = n * h * wd
    n_slabs = rows // _SLAB
    assert n_slabs * _SLAB == rows
    out = pl.pallas_call(
        _make_kernel(n_slabs, c_out),
        in_specs=[pl.BlockSpec(memory_space=pl.ANY)] * 3,
        out_specs=pl.BlockSpec(memory_space=pl.ANY),
        out_shape=jax.ShapeDtypeStruct((n_slabs, _SLAB, c_out), x.dtype),
        scratch_shapes=[
            pltpu.VMEM((n_slabs, _SLAB, c_in), x.dtype),
            pltpu.VMEM(w.shape, w.dtype),
            pltpu.VMEM(b.shape, b.dtype),
            pltpu.VMEM((8, c_out), jnp.float32),
            pltpu.SemaphoreType.DMA((_SEM_OUT + 1,)),
        ],
        compiler_params=pltpu.CompilerParams(
            vmem_limit_bytes=120 * 1024 * 1024,
            disable_bounds_checks=True,
            disable_semaphore_checks=True,
        ),
    )(x.reshape(n_slabs, _SLAB, c_in), w, b)
    return out.reshape(n, h, wd, c_out)
```

```python
import jax
import jax.numpy as jnp
import jax.experimental.pallas as pl
import jax.experimental.pallas.tpu as pltpu

_SLAB = 2048
_STREAMS = 6
_TILE = 256
_SUB = 128
_RD_STREAMS = 3
_RD_ROWS = 16
_RD_UNROLL = 2
_RD_PARTS = 2
_LEAD = 2
_TAIL = 3
_WR_ROWS = 16
_WR_UNROLL = 4
_BURST = 16
_PER_TILE = 7

_RING = 4
_SEM_LOW, _SEM_TAIL, _SEM_W, _SEM_B, _SEM_OUT = range(_RING, _RING + 5)


def _log2(n):
    assert n & (n - 1) == 0
    return n.bit_length() - 1


def _make_kernel(n_slabs, c_out):
    tiles_per_group = _SLAB // _TILE
    n_tiles = (n_slabs // _STREAMS) * tiles_per_group
    half = n_tiles // 2
    rd_rows = _RD_ROWS * _RD_UNROLL
    wr_rows = _WR_ROWS * _WR_UNROLL
    rd_chunks = _TILE // rd_rows
    wr_chunks = _TILE // wr_rows
    n_early = half - _LEAD
    rest = n_tiles * wr_chunks - _BURST - (n_tiles - n_early) * _PER_TILE
    tail_rows = _TAIL * rd_rows

    assert n_slabs % (2 * _STREAMS) == 0 and _LEAD < _RING and _LEAD < half
    assert rd_chunks % _RD_PARTS == 0 and _STREAMS % _RD_PARTS == 0
    assert _STREAMS % _RD_STREAMS == 0 and _WR_ROWS % _RD_ROWS == 0
    assert rd_chunks * rd_rows == _TILE and wr_chunks * wr_rows == _TILE
    assert rest >= 0 and 0 < _TAIL <= rd_chunks // _RD_PARTS
    assert _BURST <= n_early * wr_chunks
    for j in range(n_early, n_tiles):
        assert _BURST + (j - n_early + 1) * _PER_TILE <= (j + 1) * wr_chunks

    def window(t, row, rows):
        if isinstance(t, int):
            group = t // tiles_per_group
        else:
            group = jax.lax.shift_right_logical(t, _log2(tiles_per_group))
        start = (t & (tiles_per_group - 1)) * _TILE + row
        if not isinstance(start, int):
            start = pl.multiple_of(start, _RD_ROWS)
        return (pl.ds(group * _STREAMS, _STREAMS), pl.ds(start, rows), slice(None))

    def kernel(x_hbm, w_hbm, b_hbm, o_hbm, buf, w_v, b_v, bias_v, sem):
        def read(idx, sem_id):
            return pltpu.make_async_copy(x_hbm.at[idx], buf.at[idx], sem.at[sem_id])

        def queue_reads(t, first, stop, low_sem):
            def chunk(c, carry):
                hi = window(t, c * rd_rows, rd_rows)
                lo = window(t + half, c * rd_rows, rd_rows)
                x_hi, buf_hi, x_lo, buf_lo = (
                    x_hbm.at[hi], buf.at[hi], x_hbm.at[lo], buf.at[lo])
                for q in range(_RD_UNROLL):
                    for s in range(0, _STREAMS, _RD_STREAMS):
                        part = (pl.ds(s, _RD_STREAMS), pl.ds(q * _RD_ROWS, _RD_ROWS))
                        pltpu.make_async_copy(
                            x_hi.at[part], buf_hi.at[part], sem.at[t & (_RING - 1)]
                        ).start(priority=0)
                        pltpu.make_async_copy(
                            x_lo.at[part], buf_lo.at[part], sem.at[low_sem]
                        ).start(priority=1)
                return carry
            if stop > first:
                jax.lax.fori_loop(first, stop, chunk, 0)

        def queue_writes(first, count):
            def chunk(i, carry):
                c = first + i
                t = jax.lax.shift_right_logical(c, _log2(wr_chunks))
                idx = window(t, (c & (wr_chunks - 1)) * wr_rows, wr_rows)
                src, dst = buf.at[idx], o_hbm.at[idx]
                for q in range(_WR_UNROLL):
                    rows = (slice(None), pl.ds(q * _WR_ROWS, _WR_ROWS))
                    pltpu.make_async_copy(
                        src.at[rows], dst.at[rows], sem.at[_SEM_OUT]).start()
                return carry
            jax.lax.fori_loop(0, count, chunk, 0)

        def compute(t, first_slab, stop_slab):
            tile = buf.at[window(t, 0, _TILE)]
            for s in range(first_slab, stop_slab):
                for q in range(_TILE // _SUB):
                    rows = pl.ds(q * _SUB, _SUB)
                    acc = jnp.dot(tile[s, rows, :], w_v[0, 0],
                                  preferred_element_type=jnp.float32)
                    tile[s, rows, :] = (acc + bias_v[0:1, :]).astype(buf.dtype)

        w_copy = pltpu.make_async_copy(w_hbm, w_v, sem.at[_SEM_W])
        b_copy = pltpu.make_async_copy(b_hbm, b_v, sem.at[_SEM_B])

        w_copy.start()
        b_copy.start()

        def prologue(t, carry):
            queue_reads(t, 0, rd_chunks, _SEM_LOW)
            return carry
        jax.lax.fori_loop(0, _LEAD, prologue, 0)

        w_copy.wait()
        b_copy.wait()
        bias_v[...] = jnp.broadcast_to(
            b_v[...].astype(jnp.float32).reshape(1, c_out), bias_v.shape)

        def early(j, carry):
            read(window(j, 0, _TILE), j & (_RING - 1)).wait()
            for p in range(_RD_PARTS):
                compute(j, p * _STREAMS // _RD_PARTS, (p + 1) * _STREAMS // _RD_PARTS)
                first = p * rd_chunks // _RD_PARTS
                stop = (p + 1) * rd_chunks // _RD_PARTS
                if p < _RD_PARTS - 1:
                    queue_reads(j + _LEAD, first, stop, _SEM_LOW)
                else:
                    queue_reads(j + _LEAD, first, stop - _TAIL, _SEM_LOW)

                    @pl.when(j < n_early - 1)
                    def _():
                        queue_reads(j + _LEAD, stop - _TAIL, stop, _SEM_LOW)
            return carry
        jax.lax.fori_loop(0, n_early, early, 0)
        queue_reads(half - 1, rd_chunks - _TAIL, rd_chunks, _SEM_TAIL)

        for t in range(n_early, half):
            read(window(t, 0, _TILE), t & (_RING - 1)).wait()
        read((pl.ds(n_slabs // 2, n_slabs // 2 - _STREAMS),), _SEM_LOW).wait()
        read((pl.ds(n_slabs - _STREAMS, _STREAMS), pl.ds(0, _SLAB - tail_rows)),
             _SEM_LOW).wait()
        queue_writes(0, _BURST)
        read(window(n_tiles - 1, _TILE - tail_rows, tail_rows), _SEM_TAIL).wait()

        def late(j, carry):
            compute(j, 0, _STREAMS)
            queue_writes(_BURST + (j - n_early) * _PER_TILE, _PER_TILE)
            return carry
        jax.lax.fori_loop(n_early, n_tiles, late, 0)
        if rest:
            queue_writes(n_tiles * wr_chunks - rest, rest)
        pltpu.make_async_copy(buf, o_hbm, sem.at[_SEM_OUT]).wait()

    return kernel


@jax.jit
def pallas_standalone__standard_2d_1d_3d_conv__vision_kernel(
    x: jax.Array,
    w: jax.Array,
    b: jax.Array,
):
    n, h, wd, c_in = x.shape
    c_out = w.shape[3]
    assert w.shape[:2] == (1, 1) and c_in == c_out
    rows = n * h * wd
    n_slabs = rows // _SLAB
    assert n_slabs * _SLAB == rows
    out = pl.pallas_call(
        _make_kernel(n_slabs, c_out),
        in_specs=[pl.BlockSpec(memory_space=pl.ANY)] * 3,
        out_specs=pl.BlockSpec(memory_space=pl.ANY),
        out_shape=jax.ShapeDtypeStruct((n_slabs, _SLAB, c_out), x.dtype),
        scratch_shapes=[
            pltpu.VMEM((n_slabs, _SLAB, c_in), x.dtype),
            pltpu.VMEM(w.shape, w.dtype),
            pltpu.VMEM(b.shape, b.dtype),
            pltpu.VMEM((8, c_out), jnp.float32),
            pltpu.SemaphoreType.DMA((_SEM_OUT + 1,)),
        ],
        compiler_params=pltpu.CompilerParams(
            vmem_limit_bytes=120 * 1024 * 1024,
            disable_bounds_checks=True,
            disable_semaphore_checks=True,
        ),
    )(x.reshape(n_slabs, _SLAB, c_in), w, b)
    return out.reshape(n, h, wd, c_out)
```
